```python
import jax
import jax.numpy as jnp

def _softmax(x, axis=-1):
    return jax.nn.softmax(x, axis=axis)
def _gelu(x):
    return jax.nn.gelu(x, approximate=True)
def _silu(x):
    return jax.nn.silu(x)
def _sigmoid(x):
    return jax.nn.sigmoid(x)
def _layernorm(x, axis=-1, eps=1e-5):
    m = jnp.mean(x, axis=axis, keepdims=True)
    v = jnp.var(x, axis=axis, keepdims=True)
    return (x - m) / jnp.sqrt(v + eps)
def _scatter_add(tgt, idx, src, axis=0):
    return tgt.at[idx].add(src)
def _segment_sum(src, seg, n):
    return jax.ops.segment_sum(src, seg, n)
class _Rng:
    def __init__(self, key):
        self._k = key
    def _next(self):
        self._k, sub = jax.random.split(self._k)
        return sub
    def normal(self, shape):
        return jax.random.normal(self._next(), shape, dtype=jnp.bfloat16)
    def randint(self, lo, hi, shape):
        return jax.random.randint(self._next(), shape, lo, hi, dtype=jnp.int32)
    def uniform(self, shape, lo=0.0, hi=1.0):
        return jax.random.uniform(self._next(), shape, jnp.bfloat16, lo, hi)
    def permutation(self, n):
        return jax.random.permutation(self._next(), n)


kernel_name = 'interleave_layers__sliding_local_dilated__spectral_gfnet__prompt'

def setup_inputs():
    _rng = _Rng(jax.random.key(int.from_bytes(__import__("os").urandom(4), "little")))
    _w = (lambda a: (lambda t: t.astype(jnp.bfloat16) if jnp.issubdtype(t.dtype, jnp.floating) else t)(jnp.asarray(a)))
    def _A_setup():
        B, S, D = 1, 2048, 1024
        return {
            "x": _w((lambda *s: _rng.normal(s) * 0.05)(B, S, D)),
            "wqkv": _w((lambda *s: _rng.normal(s) * 0.05)(D, 3 * D)),
            "wo": _w((lambda *s: _rng.normal(s) * 0.05)(D, D)),
        }
    _A_in = _A_setup()

    def _B_setup():
        B, S, D = 1, 2048, 1024
        Df = D // 2 + 1
        return {
            "x": _w((lambda *s: _rng.normal(s) * 0.05)(B, S, D)),
            "w_r": _w((lambda *s: _rng.normal(s) * 0.05)(S, Df) * 0.02),
            "w_i": _w((lambda *s: _rng.normal(s) * 0.05)(S, Df) * 0.02),
        }
    _B_in = _B_setup()

    return {
        "A_x": _A_in["x"],
        "A_wqkv": _A_in["wqkv"],
        "A_wo": _A_in["wo"],
        "B_x": _B_in["x"],
        "B_w_r": _B_in["w_r"],
        "B_w_i": _B_in["w_i"],
    }

def reference(A_x, A_wqkv, A_wo, B_x, B_w_r, B_w_i):
    def _A_ref(x, wqkv, wo):
        B, S, D = x.shape
        H = 32; Dh = D // H
        W, dil = 8, 2
        qkv = (lambda x, *d: x.transpose(*d))((x @ wqkv).reshape(B, S, 3, H, Dh), 2, 0, 3, 1, 4)
        q, k, v = qkv[0], qkv[1], qkv[2]
        scale = Dh ** -0.5
        pos = jnp.arange(S)
        off = jnp.arange(W) * dil
        idx = pos[:, None] - off[None, :]
        mask = idx >= 0
        idx_c = jnp.where(mask, idx, 0).reshape(-1)
        kg = k[:, :, idx_c, :].reshape(B, H, S, W, Dh)
        vg = v[:, :, idx_c, :].reshape(B, H, S, W, Dh)
        logits = jnp.einsum("bhsd,bhswd->bhsw", q, kg) * scale
        logits = jnp.where(mask[None, None, :, :], logits, -1e9)
        attn = _softmax(logits, axis=-1)
        o = jnp.einsum("bhsw,bhswd->bhsd", attn, vg)
        return (lambda x, *d: x.transpose(*d))(o, 0, 2, 1, 3).reshape(B, S, D) @ wo

    def _B_ref(x, w_r, w_i):
        B, S, D = x.shape
        X = (lambda x, axes=(-2,-1): jnp.fft.rfft2(x.astype(jnp.float32), axes=axes))(x, axes=(-2, -1))
        W = w_r + 1j * w_i
        X = X * W
        y = (lambda x, s, axes=(-2,-1): jnp.fft.irfft2(x, s=s, axes=axes).astype(jnp.bfloat16))(X, (S, D), axes=(-2, -1))
        return y

    x = A_x
    x = x + _A_ref(_layernorm(x, axis=-1), A_wqkv, A_wo)
    x = x + _B_ref(_layernorm(x, axis=-1), B_w_r, B_w_i)
    x = x + _A_ref(_layernorm(x, axis=-1), A_wqkv, A_wo)
    x = x + _B_ref(_layernorm(x, axis=-1), B_w_r, B_w_i)
    return x
```

```python
import jax
import jax.numpy as jnp
import numpy as np
import jax.experimental.pallas as pl
import jax.experimental.pallas.tpu as pltpu

S, D, H, DH, NW = 2048, 1024, 32, 32, 8
R = 528
F32, BF16 = jnp.float32, jnp.bfloat16
G = 256


def _consts():
    n = np.arange(128)
    ms = np.zeros((16, 256, 256), np.float32)
    for n1 in range(16):
        a = -2 * np.pi * np.outer(16 * n + n1, n) / S
        c, s = np.cos(a), np.sin(a)
        ms[n1] = np.block([[c, s], [-s, c]])
    k = np.arange(64)
    fw0 = np.zeros((256, 128), np.float32)
    a = -2 * np.pi * np.outer(8 * k, n) / D
    fw0[0:64], fw0[64:128] = np.cos(a), np.sin(a)
    fw0[64] = np.cos(np.pi * n)
    a = -2 * np.pi * np.outer(8 * k + 4, n) / D
    fw0[128:192], fw0[192:256] = np.cos(a), np.sin(a)
    fw = np.zeros((3, 256, 256), np.float32)
    for r in (1, 2, 3):
        a = -2 * np.pi * np.outer(8 * k + r, n) / D
        b = -2 * np.pi * np.outer(8 * k + 8 - r, n) / D
        ca, sa, cb, sb = np.cos(a), np.sin(a), np.cos(b), np.sin(b)
        fw[r - 1] = np.block([[ca, -sa], [cb, sb], [sa, ca], [sb, -cb]])
    wt = np.full((256, 1), 2.0, np.float32)
    wt[0] = wt[64] = 1.0
    iv0 = (fw0 * wt).T
    iv = 2.0 * fw.transpose(0, 2, 1)
    dm = np.zeros((8, 256, 256), np.float32)
    dm[0, :, :128] = fw0
    dm[1:4] = fw
    dm[4, :128] = iv0
    dm[5:8] = iv
    pm = np.zeros((3, 128, 128), np.float32)
    for i in range(128):
        pm[0, (i % 16) * 8 + i // 16, i] = 1
        pm[2, (i % 8) * 16 + i // 8, i] = 1
    pm[1] = pm[0].T
    return ms.astype(BF16), dm.astype(BF16), pm.astype(BF16)


_MS, _DM, _PM = _consts()
_SLOT = {0: 0, 4: 1, 1: 2, 7: 3, 2: 4, 6: 5, 3: 6, 5: 7}


def _dot(a, b):
    return jnp.dot(a, b, preferred_element_type=F32)


def _dot_nt(a, b):
    return jax.lax.dot_general(a, b, (((1,), (1,)), ((), ())), preferred_element_type=F32)


def _fft(z, sign):
    n = len(z)
    if n == 1:
        return z
    e, o = _fft(z[0::2], sign), _fft(z[1::2], sign)
    lo, hi = [], []
    for k in range(n // 2):
        (er, ei), (pr, pi) = e[k], o[k]
        if k == 0:
            tr, ti = pr, pi
        elif 4 * k == n:
            if sign < 0:
                lo.append((er + pi, ei - pr)); hi.append((er - pi, ei + pr))
            else:
                lo.append((er - pi, ei + pr)); hi.append((er + pi, ei - pr))
            continue
        else:
            c = float(np.cos(2 * np.pi * k / n)); s = float(sign * np.sin(2 * np.pi * k / n))
            if 8 * k == n or 8 * k == 3 * n:
                if c * s > 0:
                    tr, ti = (pr - pi) * c, (pi + pr) * c
                else:
                    tr, ti = (pr + pi) * c, (pi - pr) * c
            else:
                tr, ti = pr * c - pi * s, pr * s + pi * c
        lo.append((er + tr, ei + ti)); hi.append((er - tr, ei - ti))
    return lo + hi


def _kernel(x_hbm, wqkv_hbm, wo_hbm, wr_hbm, wi_hbm, ms_hbm, dm_hbm, pm_ref, o_hbm,
            xt, xio, wst, wqt, wost, wot, wrs, wis, wrt, wit, ms, dm,
            xn, qb, kb, vb, ob, zr, zi, fr, fi, sem):
    cps = [pltpu.make_async_copy(s, d, sem.at[i]) for i, (s, d) in enumerate(
        [(x_hbm, xio), (wqkv_hbm, wst), (wo_hbm, wost), (wr_hbm, wrs), (wi_hbm, wis),
         (ms_hbm, ms), (dm_hbm, dm)])]
    for c in cps:
        c.start()

    def blk(i):
        return pl.ds(pl.multiple_of(i * 128, 128), 128)

    def load_x(tmp):
        cps[0].wait()

        @pl.loop(0, 16)
        def _(g):
            y = _dot(pm_ref[0], xio[blk(g), :])
            for n1 in range(16):
                tmp[pl.ds(pl.multiple_of(n1 * 128 + 8 * g, 8), 8), :] = y[8 * n1:8 * n1 + 8]

        @pl.loop(0, 16)
        def _(b):
            xt[:, blk(b)] = tmp[blk(b), :].T

        cps[1].wait()

        @pl.loop(0, 24)
        def _(j):
            wqt[blk(j), :] = wst[:, blk(j)].T

    pl.run_scoped(load_x, pltpu.VMEM((S, D), F32))

    def norm(b):
        v = xt[:, blk(b)]
        m = jnp.sum(v, axis=0, keepdims=True) * (1.0 / D)
        c = v - m
        var = jnp.sum(c * c, axis=0, keepdims=True) * (1.0 / D)
        return c * jax.lax.rsqrt(var + 1e-5)

    lane = jax.lax.broadcasted_iota(jnp.int32, (1, 128), 1)

    def attention():
        @pl.loop(0, 16)
        def _(b):
            xn[:, blk(b)] = norm(b).astype(BF16)

        @pl.loop(0, D // G)
        def _(g):
            r0 = pl.multiple_of(g * G, G)
            for b in range(0, 16, 4):
                rhs = xn[:, b * 128:(b + 4) * 128]
                cs = slice(b * 128, (b + 4) * 128)
                qb[:, cs] = _dot(wqt[pl.ds(r0, G), :], rhs) * (DH ** -0.5)
                for ref, off in ((kb, D), (vb, 2 * D)):
                    t = _dot(wqt[pl.ds(off + r0, G), :], rhs)
                    ref[:, (b + 16) * 128:(b + 20) * 128] = t
                    for j in range(4):
                        if b + j >= 2:
                            ref[:, (b + j) * 128:(b + j + 1) * 128] = pltpu.roll(
                                t[:, j * 128:(j + 1) * 128], 1, 1)

            @pl.loop(0, 16)
            def _(b):
                for h in range(G // DH):
                    rs = slice(h * DH, (h + 1) * DH)
                    q = qb[rs, blk(b)]
                    ls = []
                    for w in range(NW):
                        l = jnp.sum(q * kb[rs, blk(16 + b - 2 * w)], axis=0, keepdims=True)
                        if w:
                            l = jnp.where((lane == 0) & (b < 2 * w), -1e9, l)
                        ls.append(l)
                    m = ls[0]
                    for l in ls[1:]:
                        m = jnp.maximum(m, l)
                    ps = [jnp.exp(l - m) for l in ls]
                    den = ps[0]
                    for p in ps[1:]:
                        den = den + p
                    acc = ps[0] * vb[rs, blk(16 + b)]
                    for w in range(1, NW):
                        acc = acc + ps[w] * vb[rs, blk(16 + b - 2 * w)]
                    ob[pl.ds(r0 + h * DH, DH), blk(b)] = (acc / den).astype(BF16)

        @pl.loop(0, 4)
        def _(b):
            cs = pl.ds(pl.multiple_of(b * 512, 512), 512)
            xt[:, cs] += _dot(wot[...], ob[:, cs])

    c8 = float(np.sqrt(0.5))
    row0 = jax.lax.broadcasted_iota(jnp.int32, (16, 128), 0) == 0

    def spectral():
        @pl.loop(0, 16)
        def _(b):
            v = norm(b)
            x = [v[128 * j:128 * j + 128] for j in range(8)]
            a = [x[j] + x[j + 4] for j in range(4)]
            d = [x[j] - x[j + 4] for j in range(4)]
            e0, e1 = a[0] + a[2], a[1] + a[3]
            t, u = (d[1] - d[3]) * c8, (d[1] + d[3]) * c8
            ys = [(d[0] + t, -(d[2] + u)), (a[0] - a[2], a[3] - a[1]), (d[0] - t, d[2] - u)]
            y0 = _dot(dm[0, 0:128, 0:128], (e0 + e1).astype(BF16))
            y4 = _dot(dm[0, 128:256, 0:128], (e0 - e1).astype(BF16))
            zr[0:64] = y0[0:64].astype(BF16)
            zr[64:128] = y4[0:64].astype(BF16)
            zi[0:16] = jnp.where(row0, 0.0, y0[64:80]).astype(BF16)
            zi[16:64] = y0[80:128].astype(BF16)
            zi[64:128] = y4[64:128].astype(BF16)
            zr[512:R] = jnp.where(row0, y0[64:80], 0.0).astype(BF16)
            zi[512:R] = jnp.zeros((16, 128), BF16)
            for i, (yr, yi) in enumerate(ys):
                y = _dot(dm[1 + i], jnp.concatenate([yr.astype(BF16), yi.astype(BF16)], 0))
                zr[128 * (i + 1):128 * (i + 2)] = y[0:128].astype(BF16)
                zi[128 * (i + 1):128 * (i + 2)] = y[128:256].astype(BF16)
            f = _dot(jnp.concatenate([zr[...], zi[...]], 1), ms[b])
            fr[:, blk(b)] = f[:, 0:128]
            fi[:, blk(b)] = f[:, 128:256]

        @pl.loop(0, R // 8)
        def _(i):
            rs = pl.ds(pl.multiple_of(i * 8, 8), 8)
            cs = [slice(128 * j, 128 * j + 128) for j in range(16)]
            z = _fft([(fr[rs, c], fi[rs, c]) for c in cs], -1)
            p = []
            for (a, b), c in zip(z, cs):
                wr, wi = wrt[rs, c], wit[rs, c]
                p.append((a * wr - b * wi, a * wi + b * wr))
            for (a, b), c in zip(_fft(p, 1), cs):
                fr[rs, c] = a
                fi[rs, c] = b

        @pl.loop(0, 16)
        def _(b):
            f = _dot_nt(jnp.concatenate(
                [fr[:, blk(b)].astype(BF16), fi[:, blk(b)].astype(BF16)], 1), ms[b])
            re, im = f[:, 0:128], f[:, 128:256]
            im0 = jnp.where(row0, re[512:R], im[0:16])
            y0 = _dot(dm[4, 0:128, 0:128],
                      jnp.concatenate([re[0:64], im0, im[16:64]], 0).astype(BF16))
            y4 = _dot(dm[4, 0:128, 128:256],
                      jnp.concatenate([re[64:128], im[64:128]], 0).astype(BF16))
            ys = []
            for i in range(3):
                rs = slice(128 * (i + 1), 128 * (i + 2))
                y = _dot(dm[5 + i], jnp.concatenate([re[rs], im[rs]], 0).astype(BF16))
                ys.append((y[0:128], y[128:256]))
            (r1, i1), (r2, i2), (r3, i3) = ys
            e0, e1 = y0 + y4, y0 - y4
            a = [e0 + r2, e1 - i2, e0 - r2, e1 + i2]
            t, u = (r1 - r3) * c8, (i1 + i3) * c8
            d = [r1 + r3, t - u, i3 - i1, -(t + u)]
            for j in range(4):
                xt[128 * j:128 * j + 128, blk(b)] += a[j] + d[j]
                xt[128 * j + 512:128 * j + 640, blk(b)] += a[j] - d[j]

    def prep_weights():
        cps[2].wait()

        @pl.loop(0, 8)
        def _(j):
            wot[blk(j), :] = wost[:, blk(j)].T

    def prep_filter():
        for c in cps[3:]:
            c.wait()
        sc = 1.0 / (S * D)
        lane0 = jax.lax.broadcasted_iota(jnp.int32, (16, 128), 1) == 0
        sel = jnp.where(row0 & lane0, 1.0, 0.0).astype(BF16)
        first = jax.lax.broadcasted_iota(jnp.int32, (S, 128), 1) == 0
        for src, dst in ((wrs, wrt), (wis, wit)):
            for j in range(4):
                y = _dot_nt(pm_ref[2], src[:, 128 * j:128 * j + 128]) * sc
                for r in range(8):
                    o = 64 * _SLOT[r] + 16 * j
                    dst[o:o + 16, :] = y[16 * r:16 * r + 16]
            last = jnp.where(first, src[:, 512:640], jnp.zeros((S, 128), BF16))
            dst[512:R, :] = _dot_nt(sel, last) * sc

    prep_weights()
    prep_filter()

    @pl.loop(0, 2)
    def _(_):
        attention()
        spectral()

    def store_x(tmp):
        @pl.loop(0, 16)
        def _(b):
            tmp[blk(b), :] = xt[:, blk(b)].T

        @pl.loop(0, 16)
        def _(g):
            y = jnp.concatenate(
                [tmp[pl.ds(pl.multiple_of(n1 * 128 + 8 * g, 8), 8), :] for n1 in range(16)], 0)
            xio[blk(g), :] = _dot(pm_ref[1], y.astype(BF16)).astype(BF16)

        c = pltpu.make_async_copy(xio, o_hbm, sem.at[0])
        c.start()
        c.wait()

    pl.run_scoped(store_x, pltpu.VMEM((S, D), F32))


@jax.jit
def pallas_interleave_layers__sliding_local_dilated__spectral_gfnet__prompt_kernel(
    A_x: jax.Array,
    A_wqkv: jax.Array,
    A_wo: jax.Array,
    B_x: jax.Array,
    B_w_r: jax.Array,
    B_w_i: jax.Array,
):
    del B_x
    hbm = pl.BlockSpec(memory_space=pl.ANY)
    pad = ((0, 0), (0, 127))
    V = pltpu.VMEM
    out = pl.pallas_call(
        _kernel,
        in_specs=[hbm] * 7 + [pl.BlockSpec(memory_space=pltpu.VMEM)],
        out_specs=hbm,
        out_shape=jax.ShapeDtypeStruct((S, D), BF16),
        scratch_shapes=[
            V((D, S), F32), V((S, D), BF16), V((D, 3 * D), BF16), V((3 * D, D), BF16),
            V((D, D), BF16), V((D, D), BF16), V((S, 640), BF16), V((S, 640), BF16),
            V((R, S), F32), V((R, S), F32), V((16, 256, 256), BF16), V((8, 256, 256), BF16),
            V((D, S), BF16), V((G, S), F32), V((G, 2 * S), F32), V((G, 2 * S), F32),
            V((D, S), BF16), V((R, 128), BF16), V((R, 128), BF16), V((R, S), F32), V((R, S), F32),
            pltpu.SemaphoreType.DMA((7,)),
        ],
        compiler_params=pltpu.CompilerParams(vmem_limit_bytes=110 * 1024 * 1024),
    )(A_x.reshape(S, D), A_wqkv, A_wo, jnp.pad(B_w_r, pad), jnp.pad(B_w_i, pad), _MS, _DM, _PM)
    return out.reshape(1, S, D)
```

```python
import jax
import jax.numpy as jnp
import numpy as np
import jax.experimental.pallas as pl
import jax.experimental.pallas.tpu as pltpu

S, D, H, DH, NW = 2048, 1024, 32, 32, 8
R = 528
F32, BF16 = jnp.float32, jnp.bfloat16
G = 256


def _consts():
    n = np.arange(128)
    ms = np.zeros((16, 256, 256), np.float32)
    for n1 in range(16):
        a = -2 * np.pi * np.outer(16 * n + n1, n) / S
        c, s = np.cos(a), np.sin(a)
        ms[n1] = np.block([[c, s], [-s, c]])
    k = np.arange(64)
    fw0 = np.zeros((256, 128), np.float32)
    a = -2 * np.pi * np.outer(8 * k, n) / D
    fw0[0:64], fw0[64:128] = np.cos(a), np.sin(a)
    fw0[64] = np.cos(np.pi * n)
    a = -2 * np.pi * np.outer(8 * k + 4, n) / D
    fw0[128:192], fw0[192:256] = np.cos(a), np.sin(a)
    fw = np.zeros((3, 256, 256), np.float32)
    for r in (1, 2, 3):
        a = -2 * np.pi * np.outer(8 * k + r, n) / D
        b = -2 * np.pi * np.outer(8 * k + 8 - r, n) / D
        ca, sa, cb, sb = np.cos(a), np.sin(a), np.cos(b), np.sin(b)
        fw[r - 1] = np.block([[ca, -sa], [cb, sb], [sa, ca], [sb, -cb]])
    wt = np.full((256, 1), 2.0, np.float32)
    wt[0] = wt[64] = 1.0
    iv0 = (fw0 * wt).T
    iv = 2.0 * fw.transpose(0, 2, 1)
    dm = np.zeros((8, 256, 256), np.float32)
    dm[0, :, :128] = fw0
    dm[1:4] = fw
    dm[4, :128] = iv0
    dm[5:8] = iv
    pm = np.zeros((3, 128, 128), np.float32)
    for i in range(128):
        pm[0, (i % 16) * 8 + i // 16, i] = 1
        pm[2, (i % 8) * 16 + i // 8, i] = 1
    pm[1] = pm[0].T
    return ms.astype(BF16), dm.astype(BF16), pm.astype(BF16)


_MS, _DM, _PM = _consts()
_SLOT = {0: 0, 4: 1, 1: 2, 7: 3, 2: 4, 6: 5, 3: 6, 5: 7}


def _dot(a, b):
    return jnp.dot(a, b, preferred_element_type=F32)


def _dot_nt(a, b):
    return jax.lax.dot_general(a, b, (((1,), (1,)), ((), ())), preferred_element_type=F32)


def _fft(z, sign):
    n = len(z)
    if n == 1:
        return z
    e, o = _fft(z[0::2], sign), _fft(z[1::2], sign)
    lo, hi = [], []
    for k in range(n // 2):
        (er, ei), (pr, pi) = e[k], o[k]
        if k == 0:
            tr, ti = pr, pi
        elif 4 * k == n:
            if sign < 0:
                lo.append((er + pi, ei - pr)); hi.append((er - pi, ei + pr))
            else:
                lo.append((er - pi, ei + pr)); hi.append((er + pi, ei - pr))
            continue
        else:
            c = float(np.cos(2 * np.pi * k / n)); s = float(sign * np.sin(2 * np.pi * k / n))
            if 8 * k == n or 8 * k == 3 * n:
                if c * s > 0:
                    tr, ti = (pr - pi) * c, (pi + pr) * c
                else:
                    tr, ti = (pr + pi) * c, (pi - pr) * c
            else:
                tr, ti = pr * c - pi * s, pr * s + pi * c
        lo.append((er + tr, ei + ti)); hi.append((er - tr, ei - ti))
    return lo + hi


def _loop(n, name, **kw):
    def deco(f):
        with jax.named_scope("s_" + name):
            pl.loop(0, n, **kw)(f)
    return deco


def _kernel(x_hbm, wqkv_hbm, wo_hbm, wr_hbm, wi_hbm, ms_hbm, dm_hbm, pm_ref, o_hbm,
            xt, xio, wst, wqt, wost, wot, wrs, wis, wrt, wit, ms, dm,
            xn, qb, kb, vb, ob, zrs, zis, fr, fi, sem):
    cps = [pltpu.make_async_copy(s, d, sem.at[i]) for i, (s, d) in enumerate(
        [(x_hbm, xio), (wqkv_hbm, wst), (wo_hbm, wost), (wr_hbm, wrs), (wi_hbm, wis),
         (ms_hbm, ms), (dm_hbm, dm)])]
    for c in cps[:2]:
        c.start()

    def blk(i):
        return pl.ds(pl.multiple_of(i * 128, 128), 128)

    def load_x(tmp):
        cps[0].wait()

        @_loop(16, "perm")
        def _(g):
            y = _dot(pm_ref[0], xio[blk(g), :])
            for n1 in range(16):
                tmp[pl.ds(pl.multiple_of(n1 * 128 + 8 * g, 8), 8), :] = y[8 * n1:8 * n1 + 8]

        @_loop(16, "xT")
        def _(b):
            xt[:, blk(b)] = tmp[blk(b), :].T

        cps[1].wait()
        for c in cps[2:]:
            c.start()

        @_loop(24, "wqT")
        def _(j):
            wqt[blk(j), :] = wst[:, blk(j)].T

    pl.run_scoped(load_x, pltpu.VMEM((S, D), F32))

    def norm(b):
        v = xt[:, blk(b)]
        m = jnp.sum(v, axis=0, keepdims=True) * (1.0 / D)
        c = v - m
        var = jnp.sum(c * c, axis=0, keepdims=True) * (1.0 / D)
        return c * jax.lax.rsqrt(var + 1e-5)

    lane = jax.lax.broadcasted_iota(jnp.int32, (1, 128), 1)

    def attention():
        def proj(g, p, b):
            r0 = pl.multiple_of(g * G, G)
            rhs = xn[:, blk(b)]
            qb[p, :, blk(b)] = _dot(wqt[pl.ds(r0, G), :], rhs) * (DH ** -0.5)
            for ref, off in ((kb, D), (vb, 2 * D)):
                t = _dot(wqt[pl.ds(off + r0, G), :], rhs)
                ref[p, :, blk(b + 16)] = t
                ref[p, :, blk(b)] = pltpu.roll(t, 1, 1)

        def att(g, p, b):
            for h in range(G // DH):
                rs = slice(h * DH, (h + 1) * DH)
                q = qb[p, rs, blk(b)]
                ls = []
                for w in range(NW):
                    l = jnp.sum(q * kb[p, rs, blk(16 + b - 2 * w)], axis=0, keepdims=True)
                    if w:
                        l = jnp.where((lane == 0) & (b < 2 * w), -1e9, l)
                    ls.append(l)
                m = ls[0]
                for l in ls[1:]:
                    m = jnp.maximum(m, l)
                ps = [jnp.exp(l - m) for l in ls]
                den = ps[0]
                for e in ps[1:]:
                    den = den + e
                acc = ps[0] * vb[p, rs, blk(16 + b)]
                for w in range(1, NW):
                    acc = acc + ps[w] * vb[p, rs, blk(16 + b - 2 * w)]
                ob[pl.ds(pl.multiple_of(g * G, G) + h * DH, DH), blk(b)] = (acc / den).astype(BF16)

        def out(b):
            xt[:, blk(b)] += _dot(wot[...], ob[:, blk(b)])

        xn[:, 0:128] = norm(0).astype(BF16)

        @_loop(16, "ln")
        def _(b):
            proj(0, 0, b)
            nb = jnp.minimum(b + 1, 15)
            xn[:, blk(nb)] = norm(nb).astype(BF16)

        ng = D // G

        @_loop(16 * (ng - 1), "att")
        def _(i):
            g, b = i // 16, i % 16
            proj(g + 1, (g + 1) % 2, b)
            att(g, g % 2, b)

        att(ng - 1, (ng - 1) % 2, 0)

        @_loop(15, "wo")
        def _(b):
            out(b)
            att(ng - 1, (ng - 1) % 2, b + 1)

        out(15)

    c8 = float(np.sqrt(0.5))
    row0 = jax.lax.broadcasted_iota(jnp.int32, (16, 128), 0) == 0

    def spectral():
        @_loop(16, "f1", unroll=2)
        def _(b):
            zr, zi = zrs.at[b % 2], zis.at[b % 2]
            v = norm(b)
            x = [v[128 * j:128 * j + 128] for j in range(8)]
            a = [x[j] + x[j + 4] for j in range(4)]
            d = [x[j] - x[j + 4] for j in range(4)]
            e0, e1 = a[0] + a[2], a[1] + a[3]
            t, u = (d[1] - d[3]) * c8, (d[1] + d[3]) * c8
            ys = [(d[0] + t, -(d[2] + u)), (a[0] - a[2], a[3] - a[1]), (d[0] - t, d[2] - u)]
            y0 = _dot(dm[0, 0:128, 0:128], (e0 + e1).astype(BF16))
            y4 = _dot(dm[0, 128:256, 0:128], (e0 - e1).astype(BF16))
            zr[0:64] = y0[0:64].astype(BF16)
            zr[64:128] = y4[0:64].astype(BF16)
            zi[0:16] = jnp.where(row0, 0.0, y0[64:80]).astype(BF16)
            zi[16:64] = y0[80:128].astype(BF16)
            zi[64:128] = y4[64:128].astype(BF16)
            zr[512:R] = jnp.where(row0, y0[64:80], 0.0).astype(BF16)
            zi[512:R] = jnp.zeros((16, 128), BF16)
            for i, (yr, yi) in enumerate(ys):
                y = _dot(dm[1 + i], jnp.concatenate([yr.astype(BF16), yi.astype(BF16)], 0))
                zr[128 * (i + 1):128 * (i + 2)] = y[0:128].astype(BF16)
                zi[128 * (i + 1):128 * (i + 2)] = y[128:256].astype(BF16)
            f = _dot(jnp.concatenate([zr[...], zi[...]], 1), ms[b])
            fr[:, blk(b)] = f[:, 0:128]
            fi[:, blk(b)] = f[:, 128:256]

        @_loop(R // 8, "f2")
        def _(i):
            rs = pl.ds(pl.multiple_of(i * 8, 8), 8)
            cs = [slice(128 * j, 128 * j + 128) for j in range(16)]
            z = _fft([(fr[rs, c], fi[rs, c]) for c in cs], -1)
            p = []
            for (a, b), c in zip(z, cs):
                wr, wi = wrt[rs, c], wit[rs, c]
                p.append((a * wr - b * wi, a * wi + b * wr))
            for (a, b), c in zip(_fft(p, 1), cs):
                fr[rs, c] = a
                fi[rs, c] = b

        @_loop(16, "f3", unroll=2)
        def _(b):
            f = _dot_nt(jnp.concatenate(
                [fr[:, blk(b)].astype(BF16), fi[:, blk(b)].astype(BF16)], 1), ms[b])
            re, im = f[:, 0:128], f[:, 128:256]
            im0 = jnp.where(row0, re[512:R], im[0:16])
            y0 = _dot(dm[4, 0:128, 0:128],
                      jnp.concatenate([re[0:64], im0, im[16:64]], 0).astype(BF16))
            y4 = _dot(dm[4, 0:128, 128:256],
                      jnp.concatenate([re[64:128], im[64:128]], 0).astype(BF16))
            ys = []
            for i in range(3):
                rs = slice(128 * (i + 1), 128 * (i + 2))
                y = _dot(dm[5 + i], jnp.concatenate([re[rs], im[rs]], 0).astype(BF16))
                ys.append((y[0:128], y[128:256]))
            (r1, i1), (r2, i2), (r3, i3) = ys
            e0, e1 = y0 + y4, y0 - y4
            a = [e0 + r2, e1 - i2, e0 - r2, e1 + i2]
            t, u = (r1 - r3) * c8, (i1 + i3) * c8
            d = [r1 + r3, t - u, i3 - i1, -(t + u)]
            for j in range(4):
                xt[128 * j:128 * j + 128, blk(b)] += a[j] + d[j]
                xt[128 * j + 512:128 * j + 640, blk(b)] += a[j] - d[j]

    def prep_weights():
        cps[2].wait()

        @_loop(8, "woT")
        def _(j):
            wot[blk(j), :] = wost[:, blk(j)].T

    def prep_filter():
        for c in cps[3:]:
            c.wait()
        sc = 1.0 / (S * D)
        for src, dst in ((wrs, wrt), (wis, wit)):
            for j in range(4):
                y = _dot(pm_ref[2], src[128 * j:128 * j + 128, :]) * sc
                for r in range(8):
                    o = 64 * _SLOT[r] + 16 * j
                    dst[o:o + 16, :] = y[16 * r:16 * r + 16]
            dst[512:R, :] = jnp.broadcast_to(src[512:513, :].astype(F32) * sc, (16, S))

    prep_weights()

    @_loop(2, "layer")
    def _(it):
        attention()
        pl.when(it == 0)(prep_filter)
        spectral()

    def store_x(tmp):
        @_loop(16, "oT")
        def _(b):
            tmp[blk(b), :] = xt[:, blk(b)].T

        @_loop(16, "operm")
        def _(g):
            y = jnp.concatenate(
                [tmp[pl.ds(pl.multiple_of(n1 * 128 + 8 * g, 8), 8), :] for n1 in range(16)], 0)
            xio[blk(g), :] = _dot(pm_ref[1], y.astype(BF16)).astype(BF16)

        c = pltpu.make_async_copy(xio, o_hbm, sem.at[0])
        c.start()
        c.wait()

    pl.run_scoped(store_x, pltpu.VMEM((S, D), F32))


@jax.jit
def pallas_interleave_layers__sliding_local_dilated__spectral_gfnet__prompt_kernel(
    A_x: jax.Array,
    A_wqkv: jax.Array,
    A_wo: jax.Array,
    B_x: jax.Array,
    B_w_r: jax.Array,
    B_w_i: jax.Array,
):
    del B_x
    hbm = pl.BlockSpec(memory_space=pltpu.HBM)
    V = pltpu.VMEM
    out = pl.pallas_call(
        _kernel,
        in_specs=[hbm] * 7 + [pl.BlockSpec(memory_space=pltpu.VMEM)],
        out_specs=hbm,
        out_shape=jax.ShapeDtypeStruct((S, D), BF16),
        scratch_shapes=[
            V((D, S), F32), V((S, D), BF16), V((D, 3 * D), BF16), V((3 * D, D), BF16),
            V((D, D), BF16), V((D, D), BF16), V((513, S), BF16), V((513, S), BF16),
            V((R, S), F32), V((R, S), F32), V((16, 256, 256), BF16), V((8, 256, 256), BF16),
            V((D, S), BF16), V((2, G, S), F32), V((2, G, 2 * S), F32), V((2, G, 2 * S), F32),
            V((D, S), BF16), V((2, R, 128), BF16), V((2, R, 128), BF16), V((R, S), F32), V((R, S), F32),
            pltpu.SemaphoreType.DMA((7,)),
        ],
        compiler_params=pltpu.CompilerParams(vmem_limit_bytes=124 * 1024 * 1024),
    )(A_x.reshape(S, D), A_wqkv, A_wo, B_w_r.T, B_w_i.T, _MS, _DM, _PM)
    return out.reshape(1, S, D)
```

```python
import jax
import jax.numpy as jnp
import numpy as np
import jax.experimental.pallas as pl
import jax.experimental.pallas.tpu as pltpu

S, D, H, DH, NW = 2048, 1024, 32, 32, 8
R = 528
F32, BF16 = jnp.float32, jnp.bfloat16
G = 256
U = 4


def _consts():
    n = np.arange(128)
    ms = np.zeros((16, 256, 256), np.float32)
    for n1 in range(16):
        a = -2 * np.pi * np.outer(16 * n + n1, n) / S
        c, s = np.cos(a), np.sin(a)
        ms[n1] = np.block([[c, s], [-s, c]])
    k = np.arange(64)
    fw0 = np.zeros((256, 128), np.float32)
    a = -2 * np.pi * np.outer(8 * k, n) / D
    fw0[0:64], fw0[64:128] = np.cos(a), np.sin(a)
    fw0[64] = np.cos(np.pi * n)
    a = -2 * np.pi * np.outer(8 * k + 4, n) / D
    fw0[128:192], fw0[192:256] = np.cos(a), np.sin(a)
    fw = np.zeros((3, 256, 256), np.float32)
    for r in (1, 2, 3):
        a = -2 * np.pi * np.outer(8 * k + r, n) / D
        b = -2 * np.pi * np.outer(8 * k + 8 - r, n) / D
        ca, sa, cb, sb = np.cos(a), np.sin(a), np.cos(b), np.sin(b)
        fw[r - 1] = np.block([[ca, -sa], [cb, sb], [sa, ca], [sb, -cb]])
    wt = np.full((256, 1), 2.0, np.float32)
    wt[0] = wt[64] = 1.0
    iv0 = (fw0 * wt).T
    iv = 2.0 * fw.transpose(0, 2, 1)
    dm = np.zeros((8, 256, 256), np.float32)
    dm[0, :, :128] = fw0
    dm[1:4] = fw
    dm[4, :128] = iv0
    dm[5:8] = iv
    pm = np.zeros((3, 128, 128), np.float32)
    for i in range(128):
        pm[0, (i % 16) * 8 + i // 16, i] = 1
        pm[2, (i % 8) * 16 + i // 8, i] = 1
    pm[1] = pm[0].T
    return ms.astype(BF16), dm.astype(BF16), pm.astype(BF16)


_MS, _DM, _PM = _consts()
_SLOT = {0: 0, 4: 1, 1: 2, 7: 3, 2: 4, 6: 5, 3: 6, 5: 7}


def _dot(a, b):
    return jnp.dot(a, b, preferred_element_type=F32)


def _dot_nt(a, b):
    return jax.lax.dot_general(a, b, (((1,), (1,)), ((), ())), preferred_element_type=F32)


def _fft(z, sign):
    n = len(z)
    if n == 1:
        return z
    e, o = _fft(z[0::2], sign), _fft(z[1::2], sign)
    lo, hi = [], []
    for k in range(n // 2):
        (er, ei), (pr, pi) = e[k], o[k]
        if k == 0:
            tr, ti = pr, pi
        elif 4 * k == n:
            if sign < 0:
                lo.append((er + pi, ei - pr)); hi.append((er - pi, ei + pr))
            else:
                lo.append((er - pi, ei + pr)); hi.append((er + pi, ei - pr))
            continue
        else:
            c = float(np.cos(2 * np.pi * k / n)); s = float(sign * np.sin(2 * np.pi * k / n))
            if 8 * k == n or 8 * k == 3 * n:
                if c * s > 0:
                    tr, ti = (pr - pi) * c, (pi + pr) * c
                else:
                    tr, ti = (pr + pi) * c, (pi - pr) * c
            else:
                tr, ti = pr * c - pi * s, pr * s + pi * c
        lo.append((er + tr, ei + ti)); hi.append((er - tr, ei - ti))
    return lo + hi


def _loop(n, name, **kw):
    def deco(f):
        with jax.named_scope("s_" + name):
            pl.loop(0, n, **kw)(f)
    return deco


def _kernel(x_hbm, wqkv_hbm, wo_hbm, wr_hbm, wi_hbm, ms_hbm, dm_hbm, pm_ref, o_hbm,
            xt, xio, wst, wqt, wost, wot, wrs, wis, wrt, wit, ms, dm,
            xn, q0, k0, v0, q1, k1, v1, ob, zrs, zis, fr, fi, sem):
    cps = [pltpu.make_async_copy(s, d, sem.at[i]) for i, (s, d) in enumerate(
        [(x_hbm, xio), (wqkv_hbm, wst), (wo_hbm, wost), (wr_hbm, wrs), (wi_hbm, wis),
         (ms_hbm, ms), (dm_hbm, dm)])]
    for c in cps[:2]:
        c.start()

    def blk(i):
        return pl.ds(pl.multiple_of(i * 128, 128), 128)

    def wide(i):
        return pl.ds(pl.multiple_of(i * 128 * U, 128 * U), 128 * U)

    def load_x(tmp):
        cps[0].wait()

        @_loop(16, "perm")
        def _(g):
            y = _dot(pm_ref[0], xio[blk(g), :])
            for n1 in range(16):
                tmp[pl.ds(pl.multiple_of(n1 * 128 + 8 * g, 8), 8), :] = y[8 * n1:8 * n1 + 8]

        @_loop(16, "xT")
        def _(b):
            xt[:, blk(b)] = tmp[blk(b), :].T

        cps[1].wait()
        for c in cps[2:]:
            c.start()

        @_loop(24, "wqT")
        def _(j):
            wqt[blk((j % 8) // 2 * 6 + j // 8 * 2 + j % 2), :] = wst[:, blk(j)].T

    pl.run_scoped(load_x, pltpu.VMEM((S, D), F32))

    def norm(b):
        v = xt[:, blk(b)]
        m = jnp.sum(v, axis=0, keepdims=True) * (1.0 / D)
        c = v - m
        var = jnp.sum(c * c, axis=0, keepdims=True) * (1.0 / D)
        return c * jax.lax.rsqrt(var + 1e-5)

    lane = jax.lax.broadcasted_iota(jnp.int32, (1, 128), 1)

    qb, kb, vb = (q0, q1), (k0, k1), (v0, v1)

    def attention():
        def proj(g, p, b):
            y = _dot(wqt[3 * G * g:3 * G * (g + 1), :], xn[:, wide(b)])
            qb[p][:, wide(b)] = y[0:G] * float(DH ** -0.5 * np.log2(np.e))
            for ref, off in ((kb, G), (vb, 2 * G)):
                for j in range(U):
                    t = y[off:off + G, 128 * j:128 * j + 128]
                    ref[p][:, blk(U * b + j + 16)] = t
                    ref[p][:, blk(U * b + j)] = pltpu.roll(t, 1, 1)

        def att(g, p, b):
            for h in range(G // DH):
                rs = slice(h * DH, (h + 1) * DH)
                q = qb[p][rs, blk(b)]
                ls = []
                for w in range(NW):
                    l = jnp.sum(q * kb[p][rs, blk(16 + b - 2 * w)], axis=0, keepdims=True)
                    if w:
                        l = jnp.where((lane == 0) & (b < 2 * w), -1e9, l)
                    ls.append(l)
                m = ls[0]
                for l in ls[1:]:
                    m = jnp.maximum(m, l)
                ps = [jnp.exp2(l - m) for l in ls]
                den = ps[0]
                for e in ps[1:]:
                    den = den + e
                acc = ps[0] * vb[p][rs, blk(16 + b)]
                for w in range(1, NW):
                    acc = acc + ps[w] * vb[p][rs, blk(16 + b - 2 * w)]
                ob[pl.ds(g * G + h * DH, DH), blk(b)] = (acc * (1.0 / den)).astype(BF16)

        def out(b):
            xt[:, wide(b)] += _dot(wot[...], ob[:, wide(b)])

        def atts(g, b):
            for j in range(U):
                att(g, g % 2, U * b + j)

        def lns(b):
            for j in range(U):
                xn[:, blk(U * b + j)] = norm(U * b + j).astype(BF16)

        nb, ng = 16 // U, D // G
        lns(0)

        @_loop(nb - 1, "ln")
        def _(b):
            proj(0, 0, b)
            lns(b + 1)

        proj(0, 0, nb - 1)
        for g in range(ng - 1):
            @_loop(nb, "att")
            def _(b):
                proj(g + 1, (g + 1) % 2, b)
                atts(g, b)

        atts(ng - 1, 0)

        @_loop(nb - 1, "wo")
        def _(b):
            out(b)
            atts(ng - 1, b + 1)

        out(nb - 1)

    c8 = float(np.sqrt(0.5))
    row0 = jax.lax.broadcasted_iota(jnp.int32, (16, 128), 0) == 0

    def spectral():
        @_loop(16, "f1", unroll=2)
        def _(b):
            zr, zi = zrs.at[b % 2], zis.at[b % 2]
            v = norm(b)
            x = [v[128 * j:128 * j + 128] for j in range(8)]
            a = [x[j] + x[j + 4] for j in range(4)]
            d = [x[j] - x[j + 4] for j in range(4)]
            e0, e1 = a[0] + a[2], a[1] + a[3]
            t, u = (d[1] - d[3]) * c8, (d[1] + d[3]) * c8
            ys = [(d[0] + t, -(d[2] + u)), (a[0] - a[2], a[3] - a[1]), (d[0] - t, d[2] - u)]
            y0 = _dot(dm[0, 0:128, 0:128], (e0 + e1).astype(BF16))
            y4 = _dot(dm[0, 128:256, 0:128], (e0 - e1).astype(BF16))
            zr[0:64] = y0[0:64].astype(BF16)
            zr[64:128] = y4[0:64].astype(BF16)
            zi[0:16] = jnp.where(row0, 0.0, y0[64:80]).astype(BF16)
            zi[16:64] = y0[80:128].astype(BF16)
            zi[64:128] = y4[64:128].astype(BF16)
            zr[512:R] = jnp.where(row0, y0[64:80], 0.0).astype(BF16)
            zi[512:R] = jnp.zeros((16, 128), BF16)
            for i, (yr, yi) in enumerate(ys):
                y = _dot(dm[1 + i], jnp.concatenate([yr.astype(BF16), yi.astype(BF16)], 0))
                zr[128 * (i + 1):128 * (i + 2)] = y[0:128].astype(BF16)
                zi[128 * (i + 1):128 * (i + 2)] = y[128:256].astype(BF16)
            f = _dot(jnp.concatenate([zr[...], zi[...]], 1), ms[b])
            fr[:, blk(b)] = f[:, 0:128]
            fi[:, blk(b)] = f[:, 128:256]

        @_loop(R // 8, "f2")
        def _(i):
            rs = pl.ds(pl.multiple_of(i * 8, 8), 8)
            cs = [slice(128 * j, 128 * j + 128) for j in range(16)]
            z = _fft([(fr[rs, c], fi[rs, c]) for c in cs], -1)
            p = []
            for (a, b), c in zip(z, cs):
                wr, wi = wrt[rs, c], wit[rs, c]
                p.append((a * wr - b * wi, a * wi + b * wr))
            for (a, b), c in zip(_fft(p, 1), cs):
                fr[rs, c] = a
                fi[rs, c] = b

        @_loop(16, "f3", unroll=2)
        def _(b):
            f = _dot_nt(jnp.concatenate(
                [fr[:, blk(b)].astype(BF16), fi[:, blk(b)].astype(BF16)], 1), ms[b])
            re, im = f[:, 0:128], f[:, 128:256]
            im0 = jnp.where(row0, re[512:R], im[0:16])
            y0 = _dot(dm[4, 0:128, 0:128],
                      jnp.concatenate([re[0:64], im0, im[16:64]], 0).astype(BF16))
            y4 = _dot(dm[4, 0:128, 128:256],
                      jnp.concatenate([re[64:128], im[64:128]], 0).astype(BF16))
            ys = []
            for i in range(3):
                rs = slice(128 * (i + 1), 128 * (i + 2))
                y = _dot(dm[5 + i], jnp.concatenate([re[rs], im[rs]], 0).astype(BF16))
                ys.append((y[0:128], y[128:256]))
            (r1, i1), (r2, i2), (r3, i3) = ys
            e0, e1 = y0 + y4, y0 - y4
            a = [e0 + r2, e1 - i2, e0 - r2, e1 + i2]
            t, u = (r1 - r3) * c8, (i1 + i3) * c8
            d = [r1 + r3, t - u, i3 - i1, -(t + u)]
            for j in range(4):
                xt[128 * j:128 * j + 128, blk(b)] += a[j] + d[j]
                xt[128 * j + 512:128 * j + 640, blk(b)] += a[j] - d[j]

    def prep_weights():
        cps[2].wait()

        @_loop(8, "woT")
        def _(j):
            wot[blk(j), :] = wost[:, blk(j)].T

    def prep_filter():
        for c in cps[3:]:
            c.wait()
        sc = 1.0 / (S * D)
        for src, dst in ((wrs, wrt), (wis, wit)):
            for j in range(4):
                y = _dot(pm_ref[2], src[128 * j:128 * j + 128, :]) * sc
                for r in range(8):
                    o = 64 * _SLOT[r] + 16 * j
                    dst[o:o + 16, :] = y[16 * r:16 * r + 16]
            dst[512:R, :] = jnp.broadcast_to(src[512:513, :].astype(F32) * sc, (16, S))

    prep_weights()

    @_loop(2, "layer")
    def _(it):
        attention()
        pl.when(it == 0)(prep_filter)
        spectral()

    def store_x(tmp):
        @_loop(16, "oT")
        def _(b):
            tmp[blk(b), :] = xt[:, blk(b)].T

        @_loop(16, "operm")
        def _(g):
            y = jnp.concatenate(
                [tmp[pl.ds(pl.multiple_of(n1 * 128 + 8 * g, 8), 8), :] for n1 in range(16)], 0)
            xio[blk(g), :] = _dot(pm_ref[1], y.astype(BF16)).astype(BF16)

        c = pltpu.make_async_copy(xio, o_hbm, sem.at[0])
        c.start()
        c.wait()

    pl.run_scoped(store_x, pltpu.VMEM((S, D), F32))


@jax.jit
def pallas_interleave_layers__sliding_local_dilated__spectral_gfnet__prompt_kernel(
    A_x: jax.Array,
    A_wqkv: jax.Array,
    A_wo: jax.Array,
    B_x: jax.Array,
    B_w_r: jax.Array,
    B_w_i: jax.Array,
):
    del B_x
    hbm = pl.BlockSpec(memory_space=pltpu.HBM)
    V = pltpu.VMEM
    out = pl.pallas_call(
        _kernel,
        in_specs=[hbm] * 7 + [pl.BlockSpec(memory_space=pltpu.VMEM)],
        out_specs=hbm,
        out_shape=jax.ShapeDtypeStruct((S, D), BF16),
        scratch_shapes=[
            V((D, S), F32), V((S, D), BF16), V((D, 3 * D), BF16), V((3 * D, D), BF16),
            V((D, D), BF16), V((D, D), BF16), V((513, S), BF16), V((513, S), BF16),
            V((R, S), F32), V((R, S), F32), V((16, 256, 256), BF16), V((8, 256, 256), BF16),
            V((D, S), BF16), *([V((G, S), F32), V((G, 2 * S), F32), V((G, 2 * S), F32)] * 2),
            V((D, S), BF16), V((2, R, 128), BF16), V((2, R, 128), BF16), V((R, S), F32), V((R, S), F32),
            pltpu.SemaphoreType.DMA((7,)),
        ],
        compiler_params=pltpu.CompilerParams(vmem_limit_bytes=124 * 1024 * 1024),
    )(A_x.reshape(S, D), A_wqkv, A_wo, B_w_r.T, B_w_i.T, _MS, _DM, _PM)
    return out.reshape(1, S, D)
```

```python
import jax
import jax.numpy as jnp
import numpy as np
import jax.experimental.pallas as pl
import jax.experimental.pallas.tpu as pltpu

S, D, H, DH, NW = 2048, 1024, 32, 32, 8
R = 528
F32, BF16 = jnp.float32, jnp.bfloat16
G = 256
U = 4


def _consts():
    n = np.arange(128)
    ms = np.zeros((16, 256, 256), np.float32)
    for n1 in range(16):
        a = -2 * np.pi * np.outer(16 * n + n1, n) / S
        c, s = np.cos(a), np.sin(a)
        ms[n1] = np.block([[c, s], [-s, c]])
    k = np.arange(64)
    fw0 = np.zeros((256, 128), np.float32)
    a = -2 * np.pi * np.outer(8 * k, n) / D
    fw0[0:64], fw0[64:128] = np.cos(a), np.sin(a)
    fw0[64] = np.cos(np.pi * n)
    a = -2 * np.pi * np.outer(8 * k + 4, n) / D
    fw0[128:192], fw0[192:256] = np.cos(a), np.sin(a)
    fw = np.zeros((3, 256, 256), np.float32)
    for r in (1, 2, 3):
        a = -2 * np.pi * np.outer(8 * k + r, n) / D
        b = -2 * np.pi * np.outer(8 * k + 8 - r, n) / D
        ca, sa, cb, sb = np.cos(a), np.sin(a), np.cos(b), np.sin(b)
        fw[r - 1] = np.block([[ca, -sa], [cb, sb], [sa, ca], [sb, -cb]])
    wt = np.full((256, 1), 2.0, np.float32)
    wt[0] = wt[64] = 1.0
    iv0 = (fw0 * wt).T
    iv = 2.0 * fw.transpose(0, 2, 1)
    dm = np.zeros((8, 256, 256), np.float32)
    dm[0, :, :128] = fw0
    dm[1:4] = fw
    dm[4, :128] = iv0
    dm[5:8] = iv
    pm = np.zeros((3, 128, 128), np.float32)
    for i in range(128):
        pm[0, (i % 16) * 8 + i // 16, i] = 1
        pm[2, (i % 8) * 16 + i // 8, i] = 1
    pm[1] = pm[0].T
    return ms.astype(BF16), dm.astype(BF16), pm.astype(BF16)


_MS, _DM, _PM = _consts()
_SLOT = {0: 0, 4: 1, 1: 2, 7: 3, 2: 4, 6: 5, 3: 6, 5: 7}


def _dot(a, b):
    return jnp.dot(a, b, preferred_element_type=F32)


def _dot_nt(a, b):
    return jax.lax.dot_general(a, b, (((1,), (1,)), ((), ())), preferred_element_type=F32)


def _fft(z, sign):
    n = len(z)
    if n == 1:
        return z
    e, o = _fft(z[0::2], sign), _fft(z[1::2], sign)
    lo, hi = [], []
    for k in range(n // 2):
        (er, ei), (pr, pi) = e[k], o[k]
        if k == 0:
            tr, ti = pr, pi
        elif 4 * k == n:
            if sign < 0:
                lo.append((er + pi, ei - pr)); hi.append((er - pi, ei + pr))
            else:
                lo.append((er - pi, ei + pr)); hi.append((er + pi, ei - pr))
            continue
        else:
            c = float(np.cos(2 * np.pi * k / n)); s = float(sign * np.sin(2 * np.pi * k / n))
            if 8 * k == n or 8 * k == 3 * n:
                if c * s > 0:
                    tr, ti = (pr - pi) * c, (pi + pr) * c
                else:
                    tr, ti = (pr + pi) * c, (pi - pr) * c
            else:
                tr, ti = pr * c - pi * s, pr * s + pi * c
        lo.append((er + tr, ei + ti)); hi.append((er - tr, ei - ti))
    return lo + hi


def _loop(n, name, **kw):
    def deco(f):
        with jax.named_scope("s_" + name):
            pl.loop(0, n, **kw)(f)
    return deco


def _kernel(x_hbm, wqkv_hbm, wo_hbm, wr_hbm, wi_hbm, ms_hbm, dm_hbm, pm_ref, o_hbm,
            xt, xio, wst, wqt, wost, wot, wrs, wis, wrt, wit, ms, dm,
            xn, qb, kb, vb, ob, zrs, zis, fr, fi, sem):
    cps = [pltpu.make_async_copy(s, d, sem.at[i]) for i, (s, d) in enumerate(
        [(x_hbm, xio), (wqkv_hbm, wst), (wo_hbm, wost), (wr_hbm, wrs), (wi_hbm, wis),
         (ms_hbm, ms), (dm_hbm, dm)])]
    for c in cps[:1]:
        c.start()

    def blk(i):
        return pl.ds(pl.multiple_of(i * 128, 128), 128)

    def wide(i):
        return pl.ds(pl.multiple_of(i * 128 * U, 128 * U), 128 * U)

    def load_x(tmp):
        cps[0].wait()
        cps[1].start()

        @_loop(16, "perm", unroll=4)
        def _(g):
            y = _dot(pm_ref[0], xio[blk(g), :])
            for n1 in range(16):
                tmp[pl.ds(pl.multiple_of(n1 * 128 + 8 * g, 8), 8), :] = y[8 * n1:8 * n1 + 8]

        @_loop(16, "xT", unroll=4)
        def _(b):
            xt[:, blk(b)] = tmp[blk(b), :].T

        cps[1].wait()
        for c in cps[2:]:
            c.start()

        @_loop(24, "wqT", unroll=4)
        def _(j):
            wqt[blk((j % 8) // 2 * 6 + j // 8 * 2 + j % 2), :] = wst[:, blk(j)].T

    pl.run_scoped(load_x, pltpu.VMEM((S, D), F32))

    def norm(b):
        v = xt[:, blk(b)]
        m = jnp.sum(v, axis=0, keepdims=True) * (1.0 / D)
        c = v - m
        var = jnp.sum(c * c, axis=0, keepdims=True) * (1.0 / D)
        return c * jax.lax.rsqrt(var + 1e-5)

    lane = jax.lax.broadcasted_iota(jnp.int32, (1, 128), 1)

    def attention(it):
        def proj(g, p, b):
            y = _dot(wqt[pl.ds(pl.multiple_of(3 * G * g, G), 3 * G), :], xn[:, wide(b)])
            qb[p, :, wide(b)] = y[0:G] * float(DH ** -0.5 * np.log2(np.e))
            for ref, off in ((kb, G), (vb, 2 * G)):
                for j in range(U):
                    t = y[off:off + G, 128 * j:128 * j + 128]
                    ref[p, :, blk(U * b + j + 16)] = t
                    ref[p, :, blk(U * b + j)] = pltpu.roll(t, 1, 1)

        def att(g, p, b):
            for h in range(G // DH):
                rs = slice(h * DH, (h + 1) * DH)
                q = qb[p, rs, blk(b)]
                ls = []
                for w in range(NW):
                    l = jnp.sum(q * kb[p, rs, blk(16 + b - 2 * w)], axis=0, keepdims=True)
                    if w:
                        l = jnp.where((lane == 0) & (b < 2 * w), -1e9, l)
                    ls.append(l)
                m = ls[0]
                for l in ls[1:]:
                    m = jnp.maximum(m, l)
                ps = [jnp.exp2(l - m) for l in ls]
                den = ps[0]
                for e in ps[1:]:
                    den = den + e
                acc = ps[0] * vb[p, rs, blk(16 + b)]
                for w in range(1, NW):
                    acc = acc + ps[w] * vb[p, rs, blk(16 + b - 2 * w)]
                ob[pl.ds(pl.multiple_of(g * G, G) + h * DH, DH), blk(b)] = (acc * (1.0 / den)).astype(BF16)

        def out(b):
            xt[:, wide(b)] += _dot(wot[...], ob[:, wide(b)])

        def atts(g, b):
            for j in range(U):
                att(g, g % 2, U * b + j)

        def lns(b):
            for j in range(U):
                xn[:, blk(U * b + j)] = norm(U * b + j).astype(BF16)

        nb, ng = 16 // U, D // G
        lns(0)

        @_loop(nb - 1, "ln")
        def _(b):
            proj(0, 0, b)
            lns(b + 1)

        proj(0, 0, nb - 1)

        @_loop(nb * (ng - 1), "att")
        def _(i):
            g, b = i // nb, i % nb
            proj(g + 1, (g + 1) % 2, b)
            atts(g, b)

        atts(ng - 1, 0)

        @_loop(nb - 1, "wo")
        def _(b):
            out(b)
            atts(ng - 1, b + 1)

        out(nb - 1)

    c8 = float(np.sqrt(0.5))
    row0 = jax.lax.broadcasted_iota(jnp.int32, (16, 128), 0) == 0

    def spectral():
        @_loop(16, "f1", unroll=4)
        def _(b):
            zr, zi = zrs.at[b % 4], zis.at[b % 4]
            v = norm(b)
            x = [v[128 * j:128 * j + 128] for j in range(8)]
            a = [x[j] + x[j + 4] for j in range(4)]
            d = [x[j] - x[j + 4] for j in range(4)]
            e0, e1 = a[0] + a[2], a[1] + a[3]
            t, u = (d[1] - d[3]) * c8, (d[1] + d[3]) * c8
            ys = [(d[0] + t, -(d[2] + u)), (a[0] - a[2], a[3] - a[1]), (d[0] - t, d[2] - u)]
            y0 = _dot(dm[0, 0:128, 0:128], (e0 + e1).astype(BF16))
            y4 = _dot(dm[0, 128:256, 0:128], (e0 - e1).astype(BF16))
            zr[0:64] = y0[0:64].astype(BF16)
            zr[64:128] = y4[0:64].astype(BF16)
            zi[0:16] = jnp.where(row0, 0.0, y0[64:80]).astype(BF16)
            zi[16:64] = y0[80:128].astype(BF16)
            zi[64:128] = y4[64:128].astype(BF16)
            zr[512:R] = jnp.where(row0, y0[64:80], 0.0).astype(BF16)
            zi[512:R] = jnp.zeros((16, 128), BF16)
            for i, (yr, yi) in enumerate(ys):
                y = _dot(dm[1 + i], jnp.concatenate([yr.astype(BF16), yi.astype(BF16)], 0))
                zr[128 * (i + 1):128 * (i + 2)] = y[0:128].astype(BF16)
                zi[128 * (i + 1):128 * (i + 2)] = y[128:256].astype(BF16)
            f = _dot(jnp.concatenate([zr[...], zi[...]], 1), ms[b])
            fr[:, blk(b)] = f[:, 0:128]
            fi[:, blk(b)] = f[:, 128:256]

        @_loop(R // 8, "f2", unroll=2)
        def _(i):
            rs = pl.ds(pl.multiple_of(i * 8, 8), 8)
            cs = [slice(128 * j, 128 * j + 128) for j in range(16)]
            z = _fft([(fr[rs, c], fi[rs, c]) for c in cs], -1)
            p = []
            for (a, b), c in zip(z, cs):
                wr, wi = wrt[rs, c], wit[rs, c]
                p.append((a * wr - b * wi, a * wi + b * wr))
            for (a, b), c in zip(_fft(p, 1), cs):
                fr[rs, c] = a
                fi[rs, c] = b

        @_loop(16, "f3", unroll=4)
        def _(b):
            f = _dot_nt(jnp.concatenate(
                [fr[:, blk(b)].astype(BF16), fi[:, blk(b)].astype(BF16)], 1), ms[b])
            re, im = f[:, 0:128], f[:, 128:256]
            im0 = jnp.where(row0, re[512:R], im[0:16])
            y0 = _dot(dm[4, 0:128, 0:128],
                      jnp.concatenate([re[0:64], im0, im[16:64]], 0).astype(BF16))
            y4 = _dot(dm[4, 0:128, 128:256],
                      jnp.concatenate([re[64:128], im[64:128]], 0).astype(BF16))
            ys = []
            for i in range(3):
                rs = slice(128 * (i + 1), 128 * (i + 2))
                y = _dot(dm[5 + i], jnp.concatenate([re[rs], im[rs]], 0).astype(BF16))
                ys.append((y[0:128], y[128:256]))
            (r1, i1), (r2, i2), (r3, i3) = ys
            e0, e1 = y0 + y4, y0 - y4
            a = [e0 + r2, e1 - i2, e0 - r2, e1 + i2]
            t, u = (r1 - r3) * c8, (i1 + i3) * c8
            d = [r1 + r3, t - u, i3 - i1, -(t + u)]
            for j in range(4):
                xt[128 * j:128 * j + 128, blk(b)] += a[j] + d[j]
                xt[128 * j + 512:128 * j + 640, blk(b)] += a[j] - d[j]

    def prep_weights():
        cps[2].wait()

        @_loop(8, "woT", unroll=4)
        def _(j):
            wot[blk(j), :] = wost[:, blk(j)].T

    def prep_filter():
        for c in cps[3:]:
            c.wait()
        sc = 1.0 / (S * D)
        for src, dst in ((wrs, wrt), (wis, wit)):
            for j in range(4):
                y = _dot(pm_ref[2], src[128 * j:128 * j + 128, :]) * sc
                for r in range(8):
                    o = 64 * _SLOT[r] + 16 * j
                    dst[o:o + 16, :] = y[16 * r:16 * r + 16]
            dst[512:R, :] = jnp.broadcast_to(src[512:513, :].astype(F32) * sc, (16, S))


    prep_weights()

    @_loop(2, "layer")
    def _(it):
        attention(it)
        pl.when(it == 0)(prep_filter)
        spectral()

    def store_x(tmp):
        @_loop(16, "oT", unroll=4)
        def _(b):
            tmp[blk(b), :] = xt[:, blk(b)].T

        @_loop(16, "operm", unroll=4)
        def _(g):
            y = jnp.concatenate(
                [tmp[pl.ds(pl.multiple_of(n1 * 128 + 8 * g, 8), 8), :] for n1 in range(16)], 0)
            xio[blk(g), :] = _dot(pm_ref[1], y.astype(BF16)).astype(BF16)
            pltpu.make_async_copy(xio.at[blk(g)], o_hbm.at[blk(g)], sem.at[0]).start()

        pltpu.make_async_copy(xio, o_hbm, sem.at[0]).wait()

    pl.run_scoped(store_x, pltpu.VMEM((S, D), F32))


@jax.jit
def pallas_interleave_layers__sliding_local_dilated__spectral_gfnet__prompt_kernel(
    A_x: jax.Array,
    A_wqkv: jax.Array,
    A_wo: jax.Array,
    B_x: jax.Array,
    B_w_r: jax.Array,
    B_w_i: jax.Array,
):
    del B_x
    hbm = pl.BlockSpec(memory_space=pltpu.HBM)
    V = pltpu.VMEM
    out = pl.pallas_call(
        _kernel,
        in_specs=[hbm] * 7 + [pl.BlockSpec(memory_space=pltpu.VMEM)],
        out_specs=hbm,
        out_shape=jax.ShapeDtypeStruct((S, D), BF16),
        scratch_shapes=[
            V((D, S), F32), V((S, D), BF16), V((D, 3 * D), BF16), V((3 * D, D), BF16),
            V((D, D), BF16), V((D, D), BF16), V((513, S), BF16), V((513, S), BF16),
            V((R, S), F32), V((R, S), F32), V((16, 256, 256), BF16), V((8, 256, 256), BF16),
            V((D, S), BF16), V((2, G, S), F32), V((2, G, 2 * S), F32), V((2, G, 2 * S), F32),
            V((D, S), BF16), V((4, R, 128), BF16), V((4, R, 128), BF16), V((R, S), F32), V((R, S), F32),
            pltpu.SemaphoreType.DMA((7,)),
        ],
        compiler_params=pltpu.CompilerParams(vmem_limit_bytes=124 * 1024 * 1024),
    )(A_x.reshape(S, D), A_wqkv, A_wo, B_w_r.T, B_w_i.T, _MS, _DM, _PM)
    return out.reshape(1, S, D)
```

```python
import jax
import jax.numpy as jnp
import numpy as np
import jax.experimental.pallas as pl
import jax.experimental.pallas.tpu as pltpu

S, D, H, DH, NW = 2048, 1024, 32, 32, 8
R = 528
F32, BF16 = jnp.float32, jnp.bfloat16
G = 256
U = 4


def _consts():
    n = np.arange(128)
    ms = np.zeros((16, 256, 256), np.float32)
    for n1 in range(16):
        a = -2 * np.pi * np.outer(16 * n + n1, n) / S
        c, s = np.cos(a), np.sin(a)
        ms[n1] = np.block([[c, s], [-s, c]])
    k = np.arange(64)
    fw0 = np.zeros((256, 128), np.float32)
    a = -2 * np.pi * np.outer(8 * k, n) / D
    fw0[0:64], fw0[64:128] = np.cos(a), np.sin(a)
    fw0[64] = np.cos(np.pi * n)
    a = -2 * np.pi * np.outer(8 * k + 4, n) / D
    fw0[128:192], fw0[192:256] = np.cos(a), np.sin(a)
    fw = np.zeros((3, 256, 256), np.float32)
    for r in (1, 2, 3):
        a = -2 * np.pi * np.outer(8 * k + r, n) / D
        b = -2 * np.pi * np.outer(8 * k + 8 - r, n) / D
        ca, sa, cb, sb = np.cos(a), np.sin(a), np.cos(b), np.sin(b)
        fw[r - 1] = np.block([[ca, -sa], [cb, sb], [sa, ca], [sb, -cb]])
    wt = np.full((256, 1), 2.0, np.float32)
    wt[0] = wt[64] = 1.0
    iv0 = (fw0 * wt).T
    iv = 2.0 * fw.transpose(0, 2, 1)
    dm = np.zeros((8, 256, 256), np.float32)
    dm[0, :, :128] = fw0
    dm[1:4] = fw
    dm[4, :128] = iv0
    dm[5:8] = iv
    pm = np.zeros((3, 128, 128), np.float32)
    for i in range(128):
        pm[0, (i % 16) * 8 + i // 16, i] = 1
        pm[2, (i % 8) * 16 + i // 8, i] = 1
    pm[1] = pm[0].T
    return ms.astype(BF16), dm.astype(BF16), pm.astype(BF16)


_MS, _DM, _PM = _consts()
_SLOT = {0: 0, 4: 1, 1: 2, 7: 3, 2: 4, 6: 5, 3: 6, 5: 7}


def _dot(a, b):
    return jnp.dot(a, b, preferred_element_type=F32)


def _dot_nt(a, b):
    return jax.lax.dot_general(a, b, (((1,), (1,)), ((), ())), preferred_element_type=F32)


def _fft(z, sign):
    n = len(z)
    if n == 1:
        return z
    e, o = _fft(z[0::2], sign), _fft(z[1::2], sign)
    lo, hi = [], []
    for k in range(n // 2):
        (er, ei), (pr, pi) = e[k], o[k]
        if k == 0:
            tr, ti = pr, pi
        elif 4 * k == n:
            if sign < 0:
                lo.append((er + pi, ei - pr)); hi.append((er - pi, ei + pr))
            else:
                lo.append((er - pi, ei + pr)); hi.append((er + pi, ei - pr))
            continue
        else:
            c = float(np.cos(2 * np.pi * k / n)); s = float(sign * np.sin(2 * np.pi * k / n))
            if 8 * k == n or 8 * k == 3 * n:
                if c * s > 0:
                    tr, ti = (pr - pi) * c, (pi + pr) * c
                else:
                    tr, ti = (pr + pi) * c, (pi - pr) * c
            else:
                tr, ti = pr * c - pi * s, pr * s + pi * c
        lo.append((er + tr, ei + ti)); hi.append((er - tr, ei - ti))
    return lo + hi


def _loop(n, name, **kw):
    def deco(f):
        with jax.named_scope("s_" + name):
            pl.loop(0, n, **kw)(f)
    return deco


def _kernel(x_hbm, wqkv_hbm, wo_hbm, wr_hbm, wi_hbm, ms_hbm, dm_hbm, pm_ref, o_hbm,
            xt, xio, wst, wqt, wost, wot, wrs, wis, wrt, wit, ms, dm,
            xn, q0, k0, v0, q1, k1, v1, ob, zrs, zis, fr, fi, sem):
    cps = [pltpu.make_async_copy(s, d, sem.at[i]) for i, (s, d) in enumerate(
        [(x_hbm, xio), (wqkv_hbm, wst), (wo_hbm, wost), (wr_hbm, wrs), (wi_hbm, wis),
         (ms_hbm, ms), (dm_hbm, dm)])]
    for c in cps[:1]:
        c.start()

    def blk(i):
        return pl.ds(pl.multiple_of(i * 128, 128), 128)

    def wide(i):
        return pl.ds(pl.multiple_of(i * 128 * U, 128 * U), 128 * U)

    def load_x(tmp):
        cps[0].wait()
        cps[1].start()

        @_loop(16, "perm", unroll=4)
        def _(g):
            y = _dot(pm_ref[0], xio[blk(g), :])
            for n1 in range(16):
                tmp[pl.ds(pl.multiple_of(n1 * 128 + 8 * g, 8), 8), :] = y[8 * n1:8 * n1 + 8]

        @_loop(16, "xT", unroll=4)
        def _(b):
            xt[:, blk(b)] = tmp[blk(b), :].T

        cps[1].wait()
        for c in cps[2:]:
            c.start()

        @_loop(24, "wqT", unroll=4)
        def _(j):
            wqt[blk((j % 8) // 2 * 6 + j // 8 * 2 + j % 2), :] = wst[:, blk(j)].T

    pl.run_scoped(load_x, pltpu.VMEM((S, D), F32))

    def norm(b):
        v = xt[:, blk(b)]
        m = jnp.sum(v, axis=0, keepdims=True) * (1.0 / D)
        c = v - m
        var = jnp.sum(c * c, axis=0, keepdims=True) * (1.0 / D)
        return c * jax.lax.rsqrt(var + 1e-5)

    lane = jax.lax.broadcasted_iota(jnp.int32, (1, 128), 1)

    qb, kb, vb = (q0, q1), (k0, k1), (v0, v1)

    def attention(it):
        def proj(g, p, b):
            y = _dot(wqt[3 * G * g:3 * G * (g + 1), :], xn[:, wide(b)])
            qb[p][:, wide(b)] = y[0:G] * float(DH ** -0.5 * np.log2(np.e))
            for ref, off in ((kb, G), (vb, 2 * G)):
                for j in range(U):
                    t = y[off:off + G, 128 * j:128 * j + 128]
                    ref[p][:, blk(U * b + j + 16)] = t
                    ref[p][:, blk(U * b + j)] = pltpu.roll(t, 1, 1)

        def att(g, p, b):
            for h in range(G // DH):
                rs = slice(h * DH, (h + 1) * DH)
                q = qb[p][rs, blk(b)]
                ls = []
                for w in range(NW):
                    l = jnp.sum(q * kb[p][rs, blk(16 + b - 2 * w)], axis=0, keepdims=True)
                    if w:
                        l = jnp.where((lane == 0) & (b < 2 * w), -1e9, l)
                    ls.append(l)
                m = ls[0]
                for l in ls[1:]:
                    m = jnp.maximum(m, l)
                ps = [jnp.exp2(l - m) for l in ls]
                den = ps[0]
                for e in ps[1:]:
                    den = den + e
                acc = ps[0] * vb[p][rs, blk(16 + b)]
                for w in range(1, NW):
                    acc = acc + ps[w] * vb[p][rs, blk(16 + b - 2 * w)]
                ob[pl.ds(g * G + h * DH, DH), blk(b)] = (acc * (1.0 / den)).astype(BF16)

        def out(b):
            xt[:, wide(b)] += _dot(wot[...], ob[:, wide(b)])

        def atts(g, b):
            for j in range(U):
                att(g, g % 2, U * b + j)

        def lns(b):
            for j in range(U):
                xn[:, blk(U * b + j)] = norm(U * b + j).astype(BF16)

        nb, ng = 16 // U, D // G
        lns(0)

        @_loop(nb - 1, "ln")
        def _(b):
            proj(0, 0, b)
            lns(b + 1)

        proj(0, 0, nb - 1)
        for g in range(ng - 1):
            @_loop(nb, "att")
            def _(b):
                proj(g + 1, (g + 1) % 2, b)
                atts(g, b)

        atts(ng - 1, 0)

        @_loop(nb - 1, "wo")
        def _(b):
            out(b)
            atts(ng - 1, b + 1)

        out(nb - 1)

    c8 = float(np.sqrt(0.5))
    row0 = jax.lax.broadcasted_iota(jnp.int32, (16, 128), 0) == 0

    def spectral():
        @_loop(16, "f1", unroll=2)
        def _(b):
            zr, zi = zrs.at[b % 4], zis.at[b % 4]
            v = norm(b)
            x = [v[128 * j:128 * j + 128] for j in range(8)]
            a = [x[j] + x[j + 4] for j in range(4)]
            d = [x[j] - x[j + 4] for j in range(4)]
            e0, e1 = a[0] + a[2], a[1] + a[3]
            t, u = (d[1] - d[3]) * c8, (d[1] + d[3]) * c8
            ys = [(d[0] + t, -(d[2] + u)), (a[0] - a[2], a[3] - a[1]), (d[0] - t, d[2] - u)]
            y0 = _dot(dm[0, 0:128, 0:128], (e0 + e1).astype(BF16))
            y4 = _dot(dm[0, 128:256, 0:128], (e0 - e1).astype(BF16))
            zr[0:64] = y0[0:64].astype(BF16)
            zr[64:128] = y4[0:64].astype(BF16)
            zi[0:16] = jnp.where(row0, 0.0, y0[64:80]).astype(BF16)
            zi[16:64] = y0[80:128].astype(BF16)
            zi[64:128] = y4[64:128].astype(BF16)
            zr[512:R] = jnp.where(row0, y0[64:80], 0.0).astype(BF16)
            zi[512:R] = jnp.zeros((16, 128), BF16)
            for i, (yr, yi) in enumerate(ys):
                y = _dot(dm[1 + i], jnp.concatenate([yr.astype(BF16), yi.astype(BF16)], 0))
                zr[128 * (i + 1):128 * (i + 2)] = y[0:128].astype(BF16)
                zi[128 * (i + 1):128 * (i + 2)] = y[128:256].astype(BF16)
            f = _dot(jnp.concatenate([zr[...], zi[...]], 1), ms[b])
            fr[:, blk(b)] = f[:, 0:128]
            fi[:, blk(b)] = f[:, 128:256]

        @_loop(R // 8, "f2", unroll=2)
        def _(i):
            rs = pl.ds(pl.multiple_of(i * 8, 8), 8)
            cs = [slice(128 * j, 128 * j + 128) for j in range(16)]
            z = _fft([(fr[rs, c], fi[rs, c]) for c in cs], -1)
            p = []
            for (a, b), c in zip(z, cs):
                wr, wi = wrt[rs, c], wit[rs, c]
                p.append((a * wr - b * wi, a * wi + b * wr))
            for (a, b), c in zip(_fft(p, 1), cs):
                fr[rs, c] = a
                fi[rs, c] = b

        @_loop(16, "f3", unroll=2)
        def _(b):
            f = _dot_nt(jnp.concatenate(
                [fr[:, blk(b)].astype(BF16), fi[:, blk(b)].astype(BF16)], 1), ms[b])
            re, im = f[:, 0:128], f[:, 128:256]
            im0 = jnp.where(row0, re[512:R], im[0:16])
            y0 = _dot(dm[4, 0:128, 0:128],
                      jnp.concatenate([re[0:64], im0, im[16:64]], 0).astype(BF16))
            y4 = _dot(dm[4, 0:128, 128:256],
                      jnp.concatenate([re[64:128], im[64:128]], 0).astype(BF16))
            ys = []
            for i in range(3):
                rs = slice(128 * (i + 1), 128 * (i + 2))
                y = _dot(dm[5 + i], jnp.concatenate([re[rs], im[rs]], 0).astype(BF16))
                ys.append((y[0:128], y[128:256]))
            (r1, i1), (r2, i2), (r3, i3) = ys
            e0, e1 = y0 + y4, y0 - y4
            a = [e0 + r2, e1 - i2, e0 - r2, e1 + i2]
            t, u = (r1 - r3) * c8, (i1 + i3) * c8
            d = [r1 + r3, t - u, i3 - i1, -(t + u)]
            for j in range(4):
                xt[128 * j:128 * j + 128, blk(b)] += a[j] + d[j]
                xt[128 * j + 512:128 * j + 640, blk(b)] += a[j] - d[j]

    def prep_weights():
        cps[2].wait()

        @_loop(8, "woT", unroll=4)
        def _(j):
            wot[blk(j), :] = wost[:, blk(j)].T

    def prep_filter():
        for c in cps[3:]:
            c.wait()
        sc = 1.0 / (S * D)
        for src, dst in ((wrs, wrt), (wis, wit)):
            for j in range(4):
                y = _dot(pm_ref[2], src[128 * j:128 * j + 128, :]) * sc
                for r in range(8):
                    o = 64 * _SLOT[r] + 16 * j
                    dst[o:o + 16, :] = y[16 * r:16 * r + 16]
            dst[512:R, :] = jnp.broadcast_to(src[512:513, :].astype(F32) * sc, (16, S))


    prep_weights()

    @_loop(2, "layer")
    def _(it):
        attention(it)
        pl.when(it == 0)(prep_filter)
        spectral()

    def store_x(tmp):
        @_loop(16, "oT", unroll=4)
        def _(b):
            tmp[blk(b), :] = xt[:, blk(b)].T

        @_loop(16, "operm", unroll=4)
        def _(g):
            y = jnp.concatenate(
                [tmp[pl.ds(pl.multiple_of(n1 * 128 + 8 * g, 8), 8), :] for n1 in range(16)], 0)
            xio[blk(g), :] = _dot(pm_ref[1], y.astype(BF16)).astype(BF16)
            pltpu.make_async_copy(xio.at[blk(g)], o_hbm.at[blk(g)], sem.at[0]).start()

        pltpu.make_async_copy(xio, o_hbm, sem.at[0]).wait()

    pl.run_scoped(store_x, pltpu.VMEM((S, D), F32))


@jax.jit
def pallas_interleave_layers__sliding_local_dilated__spectral_gfnet__prompt_kernel(
    A_x: jax.Array,
    A_wqkv: jax.Array,
    A_wo: jax.Array,
    B_x: jax.Array,
    B_w_r: jax.Array,
    B_w_i: jax.Array,
):
    del B_x
    hbm = pl.BlockSpec(memory_space=pltpu.HBM)
    V = pltpu.VMEM
    out = pl.pallas_call(
        _kernel,
        in_specs=[hbm] * 7 + [pl.BlockSpec(memory_space=pltpu.VMEM)],
        out_specs=hbm,
        out_shape=jax.ShapeDtypeStruct((S, D), BF16),
        scratch_shapes=[
            V((D, S), F32), V((S, D), BF16), V((D, 3 * D), BF16), V((3 * D, D), BF16),
            V((D, D), BF16), V((D, D), BF16), V((513, S), BF16), V((513, S), BF16),
            V((R, S), F32), V((R, S), F32), V((16, 256, 256), BF16), V((8, 256, 256), BF16),
            V((D, S), BF16), *([V((G, S), F32), V((G, 2 * S), F32), V((G, 2 * S), F32)] * 2),
            V((D, S), BF16), V((4, R, 128), BF16), V((4, R, 128), BF16), V((R, S), F32), V((R, S), F32),
            pltpu.SemaphoreType.DMA((7,)),
        ],
        compiler_params=pltpu.CompilerParams(vmem_limit_bytes=124 * 1024 * 1024),
    )(A_x.reshape(S, D), A_wqkv, A_wo, B_w_r.T, B_w_i.T, _MS, _DM, _PM)
    return out.reshape(1, S, D)
```
